```python
import os as _os
_os.environ.setdefault('JAX_PLATFORMS', 'cpu')
import jax
import jax.numpy as jnp

def _softmax(x, axis=-1):
    return jax.nn.softmax(x, axis=axis)

def _gelu(x):
    return jax.nn.gelu(x, approximate=True)

def _silu(x):
    return jax.nn.silu(x)

def _sigmoid(x):
    return jax.nn.sigmoid(x)

def _layernorm(x, axis=-1, eps=1e-05):
    m = jnp.mean(x, axis=axis, keepdims=True)
    v = jnp.var(x, axis=axis, keepdims=True)
    return (x - m) / jnp.sqrt(v + eps)

def _scatter_add(tgt, idx, src, axis=0):
    return tgt.at[idx].add(src)

def _segment_sum(src, seg, n):
    return jax.ops.segment_sum(src, seg, n)

class _Rng:

    def __init__(self, key):
        self._k = key

    def _next(self):
        self._k, sub = jax.random.split(self._k)
        return sub

    def normal(self, shape):
        return jax.random.normal(self._next(), shape, dtype=jnp.bfloat16)

    def randint(self, lo, hi, shape):
        return jax.random.randint(self._next(), shape, lo, hi, dtype=jnp.int32)

    def uniform(self, shape, lo=0.0, hi=1.0):
        return jax.random.uniform(self._next(), shape, jnp.bfloat16, lo, hi)

    def permutation(self, n):
        return jax.random.permutation(self._next(), n)
kernel_name = 'adaLN_cond__sliding_local_dilated__mixer_channel_mlp__prompt'

def setup_inputs():
    _rng = _Rng(jax.random.key(int.from_bytes(__import__("os").urandom(4), "little")))
    _w = lambda a: (lambda t: t.astype(jnp.bfloat16) if jnp.issubdtype(t.dtype, jnp.floating) else t)(jnp.asarray(a))

    def _A_setup():
        B, S, D = (1, 2048, 512)
        return {'x': _w((lambda *s: _rng.normal(s) * 0.05)(B, S, D)), 'wqkv': _w((lambda *s: _rng.normal(s) * 0.05)(D, 3 * D)), 'wo': _w((lambda *s: _rng.normal(s) * 0.05)(D, D))}
    _A_in = _A_setup()

    def _B_setup():
        B, S, D, F = (1, 2048, 512, 1792)
        return {'x': _w((lambda *s: _rng.normal(s) * 0.05)(B, S, D)), 'w1': _w((lambda *s: _rng.normal(s) * 0.8)(D, F) * D ** (-0.5)), 'b1': _w((lambda *s: _rng.normal(s) * 0.8)(F)), 'w2': _w((lambda *s: _rng.normal(s) * 0.8)(F, D) * F ** (-0.5)), 'b2': _w((lambda *s: _rng.normal(s) * 0.4)(D))}
    _B_in = _B_setup()
    return {'A_x': _A_in['x'], 'A_wqkv': _A_in['wqkv'], 'A_wo': _A_in['wo'], 'B_x': _B_in['x'], 'B_w1': _B_in['w1'], 'B_b1': _B_in['b1'], 'B_w2': _B_in['w2'], 'B_b2': _B_in['b2'], 'c': _w((lambda *s: _rng.normal(s) * 0.05)(1, 512) * 8.0), 'w_mod': _w((lambda *s: _rng.normal(s) * 0.05)(512, 6 * 512) * 512 ** (-0.5) * 8.0)}

def reference(A_x, A_wqkv, A_wo, B_x, B_w1, B_b1, B_w2, B_b2, c, w_mod):

    def _A_ref(x, wqkv, wo):
        B, S, D = x.shape
        H = 32
        Dh = D // H
        W, dil = (8, 2)
        qkv = (lambda x, *d: x.transpose(*d))((x @ wqkv).reshape(B, S, 3, H, Dh), 2, 0, 3, 1, 4)
        q, k, v = (qkv[0], qkv[1], qkv[2])
        scale = Dh ** (-0.5)
        pos = jnp.arange(S)
        off = jnp.arange(W) * dil
        idx = pos[:, None] - off[None, :]
        mask = idx >= 0
        idx_c = jnp.where(mask, idx, 0).reshape(-1)
        kg = k[:, :, idx_c, :].reshape(B, H, S, W, Dh)
        vg = v[:, :, idx_c, :].reshape(B, H, S, W, Dh)
        logits = jnp.einsum('bhsd,bhswd->bhsw', q, kg) * scale
        logits = jnp.where(mask[None, None, :, :], logits, -1000000000.0)
        attn = _softmax(logits, axis=-1)
        o = jnp.einsum('bhsw,bhswd->bhsd', attn, vg)
        return (lambda x, *d: x.transpose(*d))(o, 0, 2, 1, 3).reshape(B, S, D) @ wo

    def _B_ref(x, w1, b1, w2, b2):
        y = _layernorm(x, axis=-1)
        h = _gelu(jnp.einsum('bsd,df->bsf', y, w1) + b1)
        return jnp.einsum('bsf,fd->bsd', h, w2) + b2
    x = A_x
    mod = (_silu(c) @ w_mod).reshape(c.shape[0], 6, 1, -1)
    sa, ca, ga, sb, cb, gb = (mod[:, 0].copy(), mod[:, 1].copy(), mod[:, 2].copy(), mod[:, 3].copy(), mod[:, 4].copy(), mod[:, 5].copy())
    h = _layernorm(x, axis=-1) * (1 + ca) + sa
    x = x + ga * _A_ref(h, A_wqkv, A_wo)
    h = _layernorm(x, axis=-1) * (1 + cb) + sb
    x = x + gb * _B_ref(h, B_w1, B_b1, B_w2, B_b2)
    return x
```

```python
import jax
import jax.numpy as jnp
import numpy as np
import jax.experimental.pallas as pl
import jax.experimental.pallas.tpu as pltpu

S, D, F, H, DH, W, DIL = 2048, 512, 1792, 32, 16, 8, 2
T = 256
RG = 16
AMODE = 'two'
OPAQUE = False
SCHED = 0
FLAGS = None
NODMA = False
HALO = 16
L = 128
KD, KF = D // L, F // L
LOG2E = 1.4426950408889634
f32, bf16, u32 = jnp.float32, jnp.bfloat16, jnp.uint32


def _cat(xs, axis=1):
    return xs[0] if len(xs) == 1 else jnp.concatenate(xs, axis=axis)


def _mean(x):
    return jnp.sum(x, axis=-1, keepdims=True) * (1.0 / D)


def _ln(x):
    xc = x - _mean(x)
    return xc * jax.lax.rsqrt(_mean(xc * xc) + 1e-5)


def _lhs7(a11, a12, a21, a22):
    return [a11 + a22, a21 + a22, a11, a22, a11 + a12, a21 - a11, a12 - a22]


def _rhs5(b11, b12, b21, b22):
    return {0: b11 + b22, 2: b12 - b22, 3: b21 - b11, 5: b11 + b12, 6: b21 + b22}


def _strassen(prod):
    m2 = prod(1)
    m4 = prod(3)
    c21 = m2 + m4
    m5 = prod(4)
    m3 = prod(2)
    c12 = m3 + m5
    m1 = prod(0)
    c11 = (m1 + (m4 - m5)) + prod(6)
    c22 = (m1 + (m3 - m2)) + prod(5)
    return c11, c12, c21, c22


def _permuted(src):
    out = [None] * 32
    for dp in range(DH // 2):
        for hp in range(2):
            a = src[pl.ds((2 * hp) * 64 + dp, 8, stride=8), :]
            b = src[pl.ds((2 * hp + 1) * 64 + dp, 8, stride=8), :]
            out[4 * dp + hp] = (a & u32(0xFFFF)) | (b << 16)
            out[4 * dp + 2 + hp] = (a >> 16) | (b & u32(0xFFFF0000))
    return jnp.concatenate(out, axis=0)


def _kernel(x_hbm, wqkv_hbm, wo_hbm, w1_hbm, b1_hbm, w2_hbm, b2_hbm, c_hbm, wm_hbm, out_hbm,
            wqkv_raw, wt_tmp, wt_v, wo_raw, wo_v, w1_raw, w1_v, w2_raw, w2_v, wm_v, b1_v, b2_v, c_v,
            par_a, par_b, b1f_v, x_v, q_v, k_v, v_v, p_v, l_v, out_v, sems, zsem):
    nb = S // T
    hf = T // 2
    sem_id = [0]
    z0 = pl.semaphore_read(zsem) if OPAQUE else 0
    zc = [0]

    def zero():
        if not OPAQUE:
            return 0
        zc[0] += 1
        return pl.multiple_of(z0 * (16 * zc[0]), 16)

    class _No:
        def wait(self):
            pass

    def dma(src, dst):
        if NODMA:
            return _No()
        cp = pltpu.make_async_copy(src, dst, sems.at[sem_id[0]])
        sem_id[0] += 1
        cp.start()
        return cp

    def wait(*groups):
        for g in groups:
            for cp in g:
                cp.wait()

    cols = lambda ref, j, n=L: ref.at[:, pl.ds(j * n, n)]
    xdma = lambda i: [dma(x_hbm.at[pl.ds(i * T, T)], x_v[i])] if i < nb else []
    mdma = lambda j: [dma(cols(wm_hbm, j, D), wm_v[j])]
    qdma = lambda p: [dma(cols(wqkv_hbm, p, D), wqkv_raw[p])]
    cp = {}
    cp['c'] = [dma(c_hbm, c_v)]
    cp['x0'] = xdma(0)
    cp['wq'] = qdma(0)
    cp['m1'] = mdma(1)
    cp['m0'] = mdma(0)
    cp['wk'] = qdma(1)
    cp['x1'] = xdma(1)
    cp['wv'] = qdma(2)
    cp['x2'] = xdma(2)
    cp['x3'] = xdma(3)
    cp['wo'] = [dma(cols(wo_hbm, j), wo_raw.at[j]) for j in range(KD)]
    cp['m234'] = mdma(2) + mdma(3) + mdma(4)
    cp['w1'] = [dma(b1_hbm, b1_v), dma(b2_hbm, b2_v)] + [dma(cols(w1_hbm, j), w1_raw.at[j]) for j in range(KF)]
    cp['w2'] = mdma(5) + [dma(cols(w2_hbm, j), w2_raw.at[j]) for j in range(KD)]
    cp['x4'] = sum([xdma(i) for i in range(4, nb)], [])

    wait(cp['c'])
    cc = c_v[...].astype(f32)
    sc = jnp.broadcast_to((cc * jax.nn.sigmoid(cc)).astype(bf16), (16, D))
    mod = lambda j: jnp.dot(sc, wm_v[j][...], preferred_element_type=f32)[:8]

    as_f32 = lambda a: pltpu.bitcast(a, bf16).astype(f32)
    as_u32 = lambda a: pltpu.bitcast(a.astype(bf16), u32)

    def store_rhs(dst, slab, b11, b12, b21, b22):
        dst[1, slab] = b11
        dst[4, slab] = b22
        for k, b in _rhs5(*[as_f32(a) for a in (b11, b12, b21, b22)]).items():
            dst[k, slab] = as_u32(b)

    def prep_qkv(p):
        wt = []
        for kc in range(KD):
            wt_tmp[p][kc] = pltpu.bitcast(wqkv_raw[p][kc * L:(kc + 1) * L, :].T, u32)
            wt.append(_permuted(wt_tmp[p].at[kc]))
        for kc in range(2):
            store_rhs(wt_v[p], kc, wt[kc][:128], wt[kc][128:], wt[kc + 2][:128], wt[kc + 2][128:])

    def prep_wo():
        w = [_permuted(wo_raw.bitcast(u32).at[j]) for j in range(KD)]
        for t in range(2):
            store_rhs(wo_v, t, w[t][:128], w[t + 2][:128], w[t][128:], w[t + 2][128:])
        par_b[0] = mod(2)
        par_b[1] = mod(3)
        par_b[2] = 1.0 + mod(4)

    def prep_w1():
        w = w1_raw.bitcast(u32)
        n = KF // 2
        for t in range(n):
            store_rhs(w1_v, t, w[t, :128], w[t + n, :128], w[t, 128:], w[t + n, 128:])
        b1f_v[...] = jnp.broadcast_to(b1_v[...].astype(f32).reshape(1, F), (8, F))

    def prep_w2():
        w = w2_raw.bitcast(u32)
        n = F // 4
        for t in range(2):
            store_rhs(w2_v, t, w[t, :n], w[t + 2, :n], w[t, n:], w[t + 2, n:])
        gb = mod(5)
        par_b[3] = 0.5 * gb
        par_b[4] = gb * b2_v[...].astype(f32).reshape(1, D)

    def par(ref, j, n=RG, cs=slice(None)):
        return _cat([ref[j, pl.ds(zero(), 8), cs]] * (n // 8), 0)

    def operands(rows):
        parts = []
        for r in range(0, hf, RG):
            u, v = rows(r), rows(hf + r)
            parts.append(_lhs7(u[:, :D // 2], u[:, D // 2:], v[:, :D // 2], v[:, D // 2:]))
        return [_cat([p[k] for p in parts], 0).astype(bf16) for k in range(7)]

    def rhs(ref, k, slabs, r0=0, n=128):
        z = zero()
        return _cat([pltpu.bitcast(ref[k, t, pl.ds(z + r0, n), :], bf16) for t in slabs])

    dot = lambda a, b: jnp.dot(a, b, preferred_element_type=f32)
    hs, os_, av, x1s, ys, gs = {}, {}, {}, {}, {}, {}

    def l1(i):
        def rows(r):
            return _ln(x_v[i][pl.ds(r, RG), :].astype(f32)) * par(par_a, 1) + par(par_a, 0)
        hs[i] = operands(rows)

    def qkv(i, p):
        nt = (((1,), (1,)), ((), ()))
        c = _strassen(lambda k: jax.lax.dot_general(hs[i][k], rhs(wt_v[p], k, (0, 1)), nt, preferred_element_type=f32))
        for half in range(2):
            for t in range(KD):
                r = c[2 * half + t // 2][:, (t % 2) * L:(t % 2 + 1) * L]
                if p == 0:
                    q_v[i][t, pl.ds(half * hf, hf), :] = r * (DH ** -0.5 * LOG2E)
                else:
                    buf = k_v if p == 1 else v_v
                    buf[i][t, pl.ds(HALO + half * hf, hf), :] = r
                    if half == 1 and i + 1 < nb:
                        buf[i + 1][t, 0:HALO, :] = r[hf - HALO:]
                    if half == 0 and i == 0:
                        buf[0][t, 0:HALO, :] = jnp.broadcast_to(r[0:1], (HALO, L))

    def att(i):
        def prod(r0):
            z = zero()
            q = [q_v[i][t, pl.ds(z + r0, RG), :] for t in range(KD)]
            ls = []
            for w in range(W):
                k = [k_v[i][t, pl.ds(z + (HALO + r0 - DIL * w), RG), :] for t in range(KD)]
                ls.append((q[0] * k[0] + q[1] * k[1]) + (q[2] * k[2] + q[3] * k[3]))
            return ls

        def rest(ls, r0):
            z = zero()
            for w in range(W):
                if i * T + r0 < DIL * w:
                    pos = r0 + jax.lax.broadcasted_iota(jnp.int32, (RG, L), 0)
                    ls[w] = jnp.where(pos >= DIL * w, ls[w], -1e9 * LOG2E)
            m = ls[0]
            for p in ls[1:]:
                m = jnp.maximum(m, p)
            es = [jnp.exp2(p - m) for p in ls]
            den = es[0]
            for e in es[1:]:
                den = den + e
            inv = 1.0 / den
            o = []
            for t in range(KD):
                acc = None
                for w in range(W):
                    term = es[w] * v_v[i][t, pl.ds(z + (HALO + r0 - DIL * w), RG), :]
                    acc = term if acc is None else acc + term
                o.append(acc * inv)
            return _cat(o)

        rot = lambda p, s: pltpu.roll(p, s, 1)
        if AMODE == 'two':
            os_[i] = operands(lambda r: rest([p + rot(p, 32) for p in [p + rot(p, 64) for p in prod(r)]], r))
        elif AMODE == 'three':
            os_[i] = operands(lambda r: rest([(p + rot(p, 64)) + (rot(p, 32) + rot(p, 96)) for p in prod(r)], r))
        else:
            lb = l_v[i % 2]
            for r in range(0, T, RG):
                for w, p in enumerate(prod(r)):
                    p = p + rot(p, 64)
                    lb[w, pl.ds(r, RG), :] = p + rot(p, 32)

            def second(r):
                z = zero()
                return rest([lb[w, pl.ds(z + r, RG), :] for w in range(W)], r)
            os_[i] = operands(second)

    def wo(i):
        c = _strassen(lambda k: dot(os_[i][k], rhs(wo_v, k, (0, 1))))
        av[i] = (_cat(c[:2]), _cat(c[2:]))

    def l2(i):
        x1s[i] = {}

        def rows(r):
            a = av[i][r // hf][r % hf:r % hf + RG]
            x1 = x_v[i][pl.ds(zero() + r, RG), :].astype(f32) + par(par_b, 0) * a
            x1s[i][r] = x1
            return _ln(_ln(x1) * par(par_b, 2) + par(par_b, 1))
        ys[i] = operands(rows)

    def w1(i):
        k1 = 0.7978845608028654

        def gelu2(r, c0):
            u = r + _cat([b1f_v[pl.ds(zero(), 8), c0:c0 + r.shape[1]]] * (hf // 8), 0)
            return u * jnp.tanh(u * (k1 + (k1 * 0.044715) * (u * u))) + u

        gs[i] = []
        for slabs in ((0, 1), (2, 3), (4, 5), (6,)):
            c = _strassen(lambda k: dot(ys[i][k], rhs(w1_v, k, slabs)))
            c0 = slabs[0] * L
            g = [gelu2(c[j], c0 + (j % 2) * (F // 2)) for j in range(4)]
            gs[i].append([a.astype(bf16) for a in _lhs7(*g)])

    out_cp = []

    def w2(i):
        def prod(k):
            acc = None
            for j, g in enumerate(gs[i]):
                r = dot(g[k], rhs(w2_v, k, (0, 1), j * L, g[k].shape[1] // 2))
                acc = r if acc is None else acc + r
            return acc
        c = _strassen(prod)
        for half in range(2):
            x1 = _cat([x1s[i][half * hf + r] for r in range(0, hf, RG)], 0)
            z = _cat(c[2 * half:2 * half + 2])
            out_v[i][pl.ds(half * hf, hf), :] = (x1 + par(par_b, 4, hf) + par(par_b, 3, hf) * z).astype(bf16)
        out_cp.append(dma(out_v[i], out_hbm.at[pl.ds(i * T, T)]))

    def run(prog):
        tasks = dict(L=l1, q=lambda i: qkv(i, 0), k=lambda i: qkv(i, 1), v=lambda i: qkv(i, 2),
                     Q=lambda i: [qkv(i, p) for p in range(3)], T=att, O=wo, N=l2, A=w1, B=w2)
        for tok in prog.split():
            if tok[0] == '!':
                wait(*[cp[n] for n in tok[1:].split(',')])
            elif tok[0] == '#':
                dict(q=lambda: prep_qkv(0), k=lambda: prep_qkv(1), v=lambda: prep_qkv(2), o=prep_wo, a=prep_w1, b=prep_w2,
                     m=lambda: par_a.__setitem__(1, 1.0 + mod(1)), s=lambda: par_a.__setitem__(0, mod(0)))[tok[1]]()
            elif int(tok[1:]) < nb:
                tasks[tok[0]](int(tok[1:]))

    pro = "!x0,wq #q !m1 #m !m0 #s L0 !wk #k q0 !x1,wv #v L1 k0 v0 T0 Q1 !x2,x3 L2 L3 T1 Q2 "
    if SCHED == 0:
        run(pro + "!wo,m234 #o T2 Q3 O0 !w1 #a N0 O1 N1 T3 A0 !w2,x4 #b L4 Q4 O2 N2 T4 B0 "
            "L5 A1 Q5 O3 N3 T5 B1 L6 A2 Q6 O4 N4 T6 B2 L7 A3 Q7 O5 N5 T7 B3 A4 O6 N6 B4 A5 O7 N7 B5 A6 A7 B6 B7")
    wait(out_cp)


@jax.jit
def pallas_adaLN_cond__sliding_local_dilated__mixer_channel_mlp__prompt_kernel(A_x, A_wqkv, A_wo, B_x, B_w1, B_b1, B_w2, B_b2, c, w_mod):
    del B_x
    vm = pltpu.VMEM
    nb = S // T
    many = lambda shape, dt, n=nb: [vm(shape, dt) for _ in range(n)]
    any_spec = pl.BlockSpec(memory_space=pl.ANY)
    out = pl.pallas_call(
        _kernel,
        in_specs=[any_spec] * 9,
        out_specs=any_spec,
        out_shape=jax.ShapeDtypeStruct((S, D), A_x.dtype),
        scratch_shapes=[
            many((D, D), bf16, 3), many((KD, D // 2, L), u32, 3), many((7, 2, D // 4, L), u32, 3),
            vm((KD, D, L), bf16), vm((7, 2, D // 4, L), u32),
            vm((KF, D, L), bf16), vm((7, KF // 2, D // 4, L), u32),
            vm((KD, F, L), bf16), vm((7, 2, F // 4, L), u32),
            many((D, D), bf16, 6), vm((F,), bf16), vm((D,), bf16), vm((1, D), bf16),
            vm((2, 8, D), f32), vm((5, 8, D), f32), vm((8, F), f32),
            many((T, D), bf16), many((KD, T, L), f32), many((KD, HALO + T, L), f32), many((KD, HALO + T, L), f32),
            many((W, T, L), f32, 2), many((W, T, L), f32, 2), many((T, D), bf16),
            pltpu.SemaphoreType.DMA((64,)), pltpu.SemaphoreType.REGULAR,
        ],
        compiler_params=pltpu.CompilerParams(vmem_limit_bytes=100 * 1024 * 1024, flags=FLAGS),
    )(A_x.reshape(S, D), A_wqkv, A_wo, B_w1, B_b1, B_w2, B_b2, c, w_mod)
    return out.reshape(A_x.shape)
```

```python
import jax
import jax.numpy as jnp
import numpy as np
import jax.experimental.pallas as pl
import jax.experimental.pallas.tpu as pltpu

S, D, F = 2048, 512, 1792
H, DH, W, DIL = 32, 16, 8, 2
T = 256
NB, HF = S // T, T // 2
RG = 16
HALO = 16
SPARE = 32
L = 128
KD, KF = D // L, F // L
MLP_GROUPS = ((0, 1), (2, 3), (4, 5), (6,))
LOG2E = 1.4426950408889634
GELU_C = 0.7978845608028654
f32, bf16, u32 = jnp.float32, jnp.bfloat16, jnp.uint32

PROG = (
    "!c !x0,wq p0 !m1 s1 M0 !m0 s0 L0 q0 !x1@4 L1 !x2@0 q1 L2 !x3@0 L3 q2 q3 !wk@5 p1 k0 !wv@5 p2 T0 v1 k1 T1 v0 k2 "
    "U0 k3 !x4,wo L4 o0 !m2,m3,m4@5 v2 s2 s3 s4 O0 U1 N0 v3 O1 N1 q4 !w1 a0 v4 A0 k4 T2 A0 A0 A0 !m5,w2 s5 b0 A1 U2 "
    "B0 A1 B0 !x5,x6,x7@3 B0 B0 A1 O2 N2 A1 B1 A2 T3 L5 A2 q5 U3 A2 T4 B1 k5 O3 B1 N3 A2 B1 U4 v5 A3 A3 B2 L6 q6 A3 "
    "O4 N4 k6 B2 A3 B2 A4 T5 v6 B2 L7 B3 U5 A4 A4 q7 O5 N5 k7 A4 B3 T6 U6 v7 B3 B3 A5 O6 B4 B4 A5 N6 A5 B4 A6 T7 A5 "
    "B5 U7 B5 B4 O7 N7 B5 A6 A6 B5 A6 A7 A7 A7 A7 B6 B6 B6 B6 B7 B7 B7 B7 "
)


def _cat(xs, axis=1):
    return xs[0] if len(xs) == 1 else jnp.concatenate(xs, axis=axis)


def _tile(t):
    return slice(t * L, (t + 1) * L)


def _rep(row, n):
    return _cat([row] * (n // 8), 0)


def _total(values):
    tiles = [v[r:r + 8, c:c + L] for v in values for r in range(0, v.shape[0], 8) for c in range(0, v.shape[1], L)]
    while len(tiles) > 1:
        tiles = [a + b for a, b in zip(tiles[::2], tiles[1::2])] + tiles[len(tiles) // 2 * 2:]
    return tiles[0]


def _zero_after(value):
    n = pltpu.bitcast(value[:8, :L], jnp.int32)[0, 0]
    return (n * (n + 1)) & 1


def _layernorm(x):
    mean = lambda a: jnp.sum(a, axis=-1, keepdims=True) * (1.0 / D)
    xc = x - mean(x)
    return xc * jnp.exp2(jnp.log(mean(xc * xc) + 1e-5) * (-0.5 * LOG2E))


def _dot(a, b, transposed=False):
    return jax.lax.dot_general(a, b, (((1,), (1 if transposed else 0,)), ((), ())), preferred_element_type=f32)


def _left_factors(a11, a12, a21, a22):
    return [a11 + a22, a21 + a22, a11, a22, a11 + a12, a21 - a11, a12 - a22]


def _right_factors(*quad):
    b11, b12, b21, b22 = [pltpu.bitcast(b, bf16).astype(f32) for b in quad]
    return [b11 + b22, quad[0], b12 - b22, b21 - b11, quad[3], b11 + b12, b21 + b22]


def _join(parts, axis):
    return [_cat([p[k] for p in parts], axis) for k in range(7)]


def _strassen_steps(prod, out, left=None, right=None, emit=lambda j, c: c):
    m2 = prod(1)
    m4 = prod(3) if left is None else prod(3) + left
    yield
    m5 = prod(4)
    out[2] = emit(2, m2 + m4)
    m1 = prod(0)
    yield
    c11 = (m1 + (m4 - m5)) + prod(6)
    yield
    m3 = prod(2) if right is None else prod(2) + right
    out[0], out[1] = emit(0, c11), emit(1, m3 + m5)
    out[3] = emit(3, ((m1 - m2) + m3) + prod(5))
    yield


def _strassen(prod, *args, **kwargs):
    out = [None] * 4
    for _ in _strassen_steps(prod, out, *args, **kwargs):
        pass
    return out


def _heads_minor(src):
    out = [None] * 32
    for dp in range(DH // 2):
        for hp in range(2):
            a = src[pl.ds((2 * hp) * 64 + dp, 8, stride=8), :]
            b = src[pl.ds((2 * hp + 1) * 64 + dp, 8, stride=8), :]
            out[4 * dp + hp] = (a & np.uint32(0xFFFF)) | (b << 16)
            out[4 * dp + 2 + hp] = (a >> 16) | (b & np.uint32(0xFFFF0000))
    return jnp.concatenate(out, axis=0)


def _kernel(x_hbm, wqkv_hbm, wo_hbm, w1_hbm, b1_hbm, w2_hbm, b2_hbm, c_hbm, wm_hbm, out_hbm,
            wqkv_v, wt_v, wo_v, w1_v, w2_v, wm_v, b1_v, b2_v, c_v,
            x_v, q_v, k_v, v_v, logit_v, hid_v, res_v, out_v, last_v, sems):
    prog = PROG.split()
    batches = [step[1:].split('@')[0].split(',') for step in prog if step[0] == '!']

    def copies(name):
        cols = lambda ref, j: ref.at[:, pl.ds(j * D, D)]
        if name[0] == 'x':
            return [(x_hbm.at[pl.ds(int(name[1]) * T, T)], x_v[int(name[1])])]
        if name[0] == 'm':
            return [(cols(wm_hbm, int(name[1])), wm_v[int(name[1])])]
        if name == 'c':
            return [(c_hbm, c_v)]
        if name == 'wo':
            return [(wo_hbm, wo_v)]
        if name == 'w1':
            return [(b1_hbm, b1_v), (b2_hbm, b2_v), (w1_hbm, w1_v)]
        if name == 'w2':
            return [(w2_hbm, w2_v)]
        p = 'qkv'.index(name[1])
        return [(cols(wqkv_hbm, p), wqkv_v[p])]

    for n, batch in enumerate(batches):
        for name in batch:
            for src, dst in copies(name):
                pltpu.make_async_copy(src, dst, sems.at[n]).start()

    marks = []

    def wait(step):
        names, _, back = step[1:].partition('@')
        n = batches.index(names.split(','))
        if marks:
            n = n + _zero_after(marks[-1 - int(back or 0)])
        for name in names.split(','):
            for src, dst in copies(name):
                pltpu.make_async_copy(src, dst, sems.at[n]).wait()

    wait(prog.pop(0))
    cond = c_v[...].astype(f32)
    silu = jnp.broadcast_to((cond * jax.nn.sigmoid(cond)).astype(bf16), (16, D))

    zero = _zero_after(jnp.broadcast_to(cond, (8, D)))
    never = jnp.full((8, L), zero, jnp.int32) != 0
    always = {n: jnp.full((n, L), zero, jnp.int32) == 0 for n in (HF, RG)}
    due, small, sent, sends = [], [], [], []

    def store(view, val):
        pltpu.store(view, val, mask=_cat([always[val.shape[0]]] * (val.shape[1] // L)))

    def kept(view, val):
        store(view, val)
        return view[...]

    def tied(w, token):
        tail = jnp.where(never, pltpu.bitcast(token, w.dtype), w[-8:, -L:])
        return _cat([w[:, :-L], _cat([w[:-8, -L:], tail], 0)])

    def dot(a, w, transposed=False):
        if due:
            token = due.pop(0)[1]
            w = tied(w, token[:8] + token[8:])
        marks.append(_dot(a, pltpu.bitcast(w, bf16) if w.dtype == u32 else w.astype(bf16), transposed))
        if small:
            small.pop(0)()
        return marks[-1]

    def send(ref, dst):
        sends.append(pltpu.make_async_copy(ref.at[pl.ds(0, ref.shape[0] - SPARE)], dst, sems.at[len(batches)]))
        sends[-1].start()
        sent.append(ref)

    def after_sends(w):
        while sent:
            ref = sent.pop()
            spare = ref.shape[0] - SPARE
            ref[pl.ds(pl.multiple_of(spare + 16 * zero, 16), 16), :] = jnp.zeros((16, ref.shape[1]), bf16)
            w = tied(w, pltpu.bitcast(ref[spare:spare + 16, :L], u32))
        return w

    mods, bias, wts = {}, {}, {}

    def mod(j):
        while j not in mods:
            small.pop(0)()
        return mods[j]

    def modulation(j):
        parts = []

        def one():
            parts.append(_dot(silu, wm_v[j][:, _tile(len(parts))])[:8])
            if len(parts) == KD:
                m = _cat(parts)
                mods[j] = 1.0 + m if j in (1, 4) else 0.5 * m if j == 5 else m
        small.extend([one] * KD)
        if j < 2:
            marks.append(mod(j))

    def prep_qkv(p):
        wt = []
        for kc in range(KD):
            wt_v[p][kc] = pltpu.bitcast(wqkv_v[p][kc * L:(kc + 1) * L, :].T, u32)
            wt.append(_heads_minor(wt_v[p].at[kc]))
        wts['qkv', p] = _join([_right_factors(wt[kc][:L], wt[kc][L:], wt[kc + 2][:L], wt[kc + 2][L:]) for kc in range(2)], 1)
        if not marks:
            marks.append(_total([wts['qkv', p][k] for k in (0, 2, 3, 5, 6)]))

    def prep_wo(_):
        for t in range(KD):
            wt_v[3][t] = pltpu.bitcast(wo_v[:, _tile(t)], u32)
        w = [_heads_minor(wt_v[3].at[t]) for t in range(KD)]
        wts['o'] = _join([_right_factors(w[t][:L], w[t + 2][:L], w[t][L:], w[t + 2][L:]) for t in range(2)], 1)

    def prep_w1(_):
        w, n = lambda t, r: pltpu.bitcast(w1_v[r:r + 2 * L, _tile(t)], u32), KF // 2
        for gi, tiles in enumerate(MLP_GROUPS):
            wts[1, gi] = _join([_right_factors(w(t, 0), w(t + n, 0), w(t, 2 * L), w(t + n, 2 * L)) for t in tiles], 1)
        bias[1] = jnp.broadcast_to(b1_v[...].astype(f32).reshape(1, F), (8, F))

    def prep_w2(_):
        w, n = lambda t, a, b: pltpu.bitcast(w2_v[2 * a:2 * b, _tile(t)], u32), F // 4
        for gi, tiles in enumerate(MLP_GROUPS):
            a, b = tiles[0] * L // 2, (tiles[-1] + 1) * L // 2
            wts[2, gi] = _join([_right_factors(w(t, a, b), w(t + 2, a, b), w(t, n + a, n + b), w(t + 2, n + a, n + b))
                                for t in range(2)], 1)
        bias[2] = jnp.broadcast_to(2.0 * b2_v[...].astype(f32).reshape(1, D), (8, D))

    scaled, normed, attended, mixed, resid, mlp_in, hidden = {}, {}, {}, {}, {}, {}, {}

    def factors(rows):
        parts = []
        for r in range(0, HF, RG):
            u, v = rows(r), rows(HF + r)
            parts.append(_left_factors(u[:, :D // 2], u[:, D // 2:], v[:, :D // 2], v[:, D // 2:]))
        return [a.astype(bf16) for a in _join(parts, 0)]

    x_rows = lambda i, r: x_v[i][pl.ds(r, RG), :].astype(f32)
    scale_rows = lambda i, r: _layernorm(x_rows(i, r)) * _rep(mod(1), RG)

    def scale_early(i):
        for r in range(0, T, RG):
            scaled[i, r] = scale_rows(i, r)
        marks.append(_total([scaled[i, r] for r in range(0, T, RG)]))

    def input_norm(i):
        normed[i] = factors(lambda r: (scaled[i, r] if (i, r) in scaled else scale_rows(i, r)) + _rep(mod(0), RG))

    def project(i, p):
        def emit(j, c):
            half = j // 2
            for tt in range(2):
                t, r = 2 * (j % 2) + tt, c[:, tt * L:(tt + 1) * L]
                if p == 0:
                    store(q_v[i].at[t, pl.ds(half * HF, HF), :], r * (DH ** -0.5 * LOG2E))
                    continue
                buf = k_v if p == 1 else v_v
                store(buf[i].at[t, pl.ds(HALO + half * HF, HF), :], r)
                if half == 1 and i + 1 < NB:
                    store(buf[i + 1].at[t, pl.ds(0, HALO), :], r[HF - HALO:])
                if half == 0 and i == 0:
                    store(buf[0].at[t, pl.ds(0, HALO), :], jnp.broadcast_to(r[0:1], (HALO, L)))
        _strassen(lambda k: dot(normed[i][k], wts['qkv', p][k], True), emit=emit)

    window = lambda ref, t, r, w: ref[t, pl.ds(HALO + r - DIL * w, RG), :]

    def logits(i):
        for r in range(0, T, RG):
            q = [q_v[i][t, pl.ds(r, RG), :] for t in range(KD)]
            for w in range(W):
                k = [window(k_v[i], t, r, w) for t in range(KD)]
                p = (q[0] * k[0] + q[1] * k[1]) + (q[2] * k[2] + q[3] * k[3])
                p = (p + pltpu.roll(p, 2 * H, 1)) + (pltpu.roll(p, H, 1) + pltpu.roll(p, 3 * H, 1))
                store(logit_v[i].at[w, pl.ds(r, RG), :], p)

    def attend(i):
        def rows(r):
            ls = [logit_v[i][w, pl.ds(r, RG), :] for w in range(W)]
            for w in range(W):
                if i * T + r < DIL * w:
                    pos = r + jax.lax.broadcasted_iota(jnp.int32, (RG, L), 0)
                    ls[w] = jnp.where(pos >= DIL * w, ls[w], -1e9 * LOG2E)
            top = ls[0]
            for p in ls[1:]:
                top = jnp.maximum(top, p)
            den, acc = None, [None] * KD
            for w in range(W):
                e = jnp.exp2(ls[w] - top)
                den = e if w == 0 else den + e
                for t in range(KD):
                    term = e * window(v_v[i], t, r, w)
                    acc[t] = term if w == 0 else acc[t] + term
            inv = pl.reciprocal(den, approx=True)
            inv = inv * (2.0 - den * inv)
            o = [a * inv for a in acc]
            due.append((i, o[1] + o[3]))
            return _cat(o)
        attended[i] = factors(rows)

    def out_proj(i):
        due[:] = [d for d in due if d[0] != i]
        c = _strassen(lambda k: dot(attended[i][k], wts['o'][k]))
        mixed[i] = (_cat(c[:2]), _cat(c[2:]))

    def mlp_norm(i):
        def rows(r):
            x = x_rows(i, r) + _rep(mod(2), RG) * mixed[i][r // HF][r % HF:r % HF + RG]
            resid[i, r] = x = kept(res_v[i].at[pl.ds(r, RG)], x)
            return _layernorm(_layernorm(x) * _rep(mod(4), RG) + _rep(mod(3), RG))
        mlp_in[i] = factors(rows)

    def mlp_up(i):
        for gi, tiles in enumerate(MLP_GROUPS):
            c0, n = tiles[0] * L, len(tiles) * L
            prod = lambda k: dot(mlp_in[i][k], after_sends(wts[1, gi][k]) if (gi, k) == (1, 1) else wts[1, gi][k])
            c = _strassen(prod, *[_rep(bias[1][:, s:s + n], HF) for s in (c0, F // 2 + c0)])
            g = [u * jnp.tanh(u * (GELU_C + (GELU_C * 0.044715) * (u * u))) + u for u in c]
            g = [kept(hid_v[i].at[j, :, pl.ds(c0, n)], a) for j, a in enumerate(g)]
            hidden[i, gi] = [a.astype(bf16) for a in _left_factors(*g)]
            yield

    def mlp_down(i):
        def prod(k):
            acc = None
            for gi in range(len(MLP_GROUPS)):
                last = (i, gi) == (NB - 1, len(MLP_GROUPS) - 1)
                r = dot(hidden[i, gi][k], after_sends(wts[2, gi][k]) if last else wts[2, gi][k])
                acc = r if acc is None else acc + r
            return acc

        def emit(j, c):
            r0, c0, n = (j // 2) * HF, (j % 2) * D // 2, D // 2
            x = _cat([resid[i, r0 + r][:, c0:c0 + n] for r in range(0, HF, RG)], 0)
            val = (x + _rep(mod(5)[:, c0:c0 + n], HF) * c).astype(bf16)
            if i == NB - 1:
                last_v[j][0:HF, :] = val
                send(last_v[j], out_hbm.at[pl.ds(i * T + r0, HF), pl.ds(c0, n)])
            else:
                out_v[i][pl.ds(r0, HF), pl.ds(c0, n)] = val
                if j == 3:
                    send(out_v[i], out_hbm.at[pl.ds(i * T, T)])
        yield from _strassen_steps(prod, [None] * 4, _rep(bias[2][:, :D // 2], HF), _rep(bias[2][:, D // 2:], HF), emit)

    up, down = [mlp_up(i) for i in range(NB)], [mlp_down(i) for i in range(NB)]
    steps = dict(s=modulation, p=prep_qkv, o=prep_wo, a=prep_w1, b=prep_w2, M=scale_early, L=input_norm,
                 q=lambda i: project(i, 0), k=lambda i: project(i, 1), v=lambda i: project(i, 2),
                 T=logits, U=attend, O=out_proj, N=mlp_norm, A=lambda i: next(up[i]), B=lambda i: next(down[i]))
    for step in prog:
        if step[0] == '!':
            wait(step)
        else:
            steps[step[0]](int(step[1:]))
    for copy in sends:
        copy.wait()


@jax.jit
def pallas_adaLN_cond__sliding_local_dilated__mixer_channel_mlp__prompt_kernel(
    A_x: jax.Array,
    A_wqkv: jax.Array,
    A_wo: jax.Array,
    B_x: jax.Array,
    B_w1: jax.Array,
    B_b1: jax.Array,
    B_w2: jax.Array,
    B_b2: jax.Array,
    c: jax.Array,
    w_mod: jax.Array,
):
    del B_x
    vm = pltpu.VMEM
    many = lambda shape, dtype, n=NB: [vm(shape, dtype) for _ in range(n)]
    in_hbm = pl.BlockSpec(memory_space=pl.ANY)
    out = pl.pallas_call(
        _kernel,
        in_specs=[in_hbm] * 9,
        out_specs=in_hbm,
        out_shape=jax.ShapeDtypeStruct((S, D), A_x.dtype),
        scratch_shapes=[
            many((D, D), bf16, 3), many((KD, D // 2, L), u32, 4),
            vm((D, D), bf16), vm((D, F), bf16), vm((F, D), bf16),
            many((D, D), bf16, 6), vm((F,), bf16), vm((D,), bf16), vm((1, D), bf16),
            many((T, D), bf16), many((KD, T, L), f32), many((KD, HALO + T, L), f32), many((KD, HALO + T, L), f32),
            many((W, T, L), f32), many((4, HF, F // 2), f32), many((T, D), f32),
            many((T + SPARE, D), bf16, NB - 1), many((HF + SPARE, D // 2), bf16, 4),
            pltpu.SemaphoreType.DMA((PROG.count('!') + 1,)),
        ],
        compiler_params=pltpu.CompilerParams(
            vmem_limit_bytes=100 * 1024 * 1024,
            flags={'XLA_TPU_RESCHEDULE_DMA_DONES': True},
            disable_semaphore_checks=True,
        ),
    )(A_x.reshape(S, D), A_wqkv, A_wo, B_w1, B_b1, B_w2, B_b2, c, w_mod)
    return out.reshape(A_x.shape)
```
